```python
import os as _os
_os.environ.setdefault("JAX_PLATFORMS", "cpu")
import jax
import jax.numpy as jnp

def _softmax(x, axis=-1):
    return jax.nn.softmax(x, axis=axis)
def _gelu(x):
    return jax.nn.gelu(x, approximate=True)
def _silu(x):
    return jax.nn.silu(x)
def _sigmoid(x):
    return jax.nn.sigmoid(x)
def _layernorm(x, axis=-1, eps=1e-5):
    m = jnp.mean(x, axis=axis, keepdims=True)
    v = jnp.var(x, axis=axis, keepdims=True)
    return (x - m) / jnp.sqrt(v + eps)
def _scatter_add(tgt, idx, src, axis=0):
    return tgt.at[idx].add(src)
def _segment_sum(src, seg, n):
    return jax.ops.segment_sum(src, seg, n)
class _Rng:
    def __init__(self, key):
        self._k = key
    def _next(self):
        self._k, sub = jax.random.split(self._k)
        return sub
    def normal(self, shape):
        return jax.random.normal(self._next(), shape, dtype=jnp.bfloat16)
    def randint(self, lo, hi, shape):
        return jax.random.randint(self._next(), shape, lo, hi, dtype=jnp.int32)
    def uniform(self, shape, lo=0.0, hi=1.0):
        return jax.random.uniform(self._next(), shape, jnp.bfloat16, lo, hi)
    def permutation(self, n):
        return jax.random.permutation(self._next(), n)


kernel_name = 'concat_heads__ssm_conv_s4__linear_attn_block__prompt'

def setup_inputs():
    _rng = _Rng(jax.random.key(int.from_bytes(__import__("os").urandom(4), "little")))
    _w = (lambda a: (lambda t: t.astype(jnp.bfloat16) if jnp.issubdtype(t.dtype, jnp.floating) else t)(jnp.asarray(a)))
    def _A_setup():
        B, L, D, N = 1, 2048, 512, 128
        A_re = -jnp.exp((lambda *s: _rng.normal(s) * 0.1)(D, N))
        A_im = jnp.pi * (lambda *s: _rng.normal(s) * 0.1)(D, N)
        B_re = (lambda *s: _rng.normal(s) * 0.1)(D, N)
        B_im = (lambda *s: _rng.normal(s) * 0.1)(D, N)
        C_re = (lambda *s: _rng.normal(s) * 0.1)(D, N)
        C_im = (lambda *s: _rng.normal(s) * 0.1)(D, N)
        log_dt = (lambda *s: _rng.normal(s) * 0.1)(D) * 0.5 - 4.0
        Dskip = (lambda *s: _rng.normal(s) * 0.05)(D)
        return {
            "u": _w((lambda *s: _rng.normal(s) * 0.05)(B, L, D)),
            "A_re": _w(A_re),
            "A_im": _w(A_im),
            "B_re": _w(B_re),
            "B_im": _w(B_im),
            "C_re": _w(C_re),
            "C_im": _w(C_im),
            "log_dt": _w(log_dt),
            "Dskip": _w(Dskip),
        }
    _A_in = _A_setup()

    def _B_setup():
        B, S, D = 1, 2048, 512
        return {
            "x": _w((lambda *s: _rng.normal(s) * 0.05)(B, S, D)),
            "wqkv": _w((lambda *s: _rng.normal(s) * 0.4)(D, 3 * D)),
            "wo": _w((lambda *s: _rng.normal(s) * 0.05)(D, D)),
        }
    _B_in = _B_setup()

    return {
        "A_u": _A_in["u"],
        "A_A_re": _A_in["A_re"],
        "A_A_im": _A_in["A_im"],
        "A_B_re": _A_in["B_re"],
        "A_B_im": _A_in["B_im"],
        "A_C_re": _A_in["C_re"],
        "A_C_im": _A_in["C_im"],
        "A_log_dt": _A_in["log_dt"],
        "A_Dskip": _A_in["Dskip"],
        "B_x": _B_in["x"],
        "B_wqkv": _B_in["wqkv"],
        "B_wo": _B_in["wo"],
    }

def reference(A_u, A_A_re, A_A_im, A_B_re, A_B_im, A_C_re, A_C_im, A_log_dt, A_Dskip, B_x, B_wqkv, B_wo):
    def _A_ref(u, A_re, A_im, B_re, B_im, C_re, C_im, log_dt, Dskip):
        Bsz, L, D = u.shape
        dt = jnp.exp(log_dt)[:, None]
        A = A_re + 1j * A_im
        Bc = B_re + 1j * B_im
        Cc = C_re + 1j * C_im
        logdA = dt * A
        dB = dt * Bc
        l = (lambda x, dt: x.astype(dt))(jnp.arange(L), A_re.dtype)
        P = jnp.exp(logdA[:, :, None] * l[None, None, :])
        K = jnp.einsum("dn,dnl,dn->dl", Cc, P, dB).real
        L2 = 2 * L
        Kp = jnp.pad(K, ((0, 0), (0, L)))
        up = (lambda x, *d: x.transpose(*d))(u, 0, 2, 1)
        up = jnp.pad(up, ((0, 0), (0, 0), (0, L)))
        Kf = (lambda x, axes=(-2,-1): jnp.fft.rfft2(x.astype(jnp.float32), axes=axes))(Kp[:, None, :], axes=(-2, -1))
        Uf = (lambda x, axes=(-2,-1): jnp.fft.rfft2(x.astype(jnp.float32), axes=axes))(up[:, :, None, :], axes=(-2, -1))
        Yf = Uf * Kf[None, :, :, :]
        y = (lambda x, s, axes=(-2,-1): jnp.fft.irfft2(x, s=s, axes=axes).astype(jnp.bfloat16))(Yf, (1, L2), axes=(-2, -1))[:, :, 0, :L]
        y = (lambda x, *d: x.transpose(*d))(y, 0, 2, 1) + u * Dskip[None, None, :]
        return y

    def _B_ref(x, wqkv, wo):
        B, S, D = x.shape
        H = 32; Dh = D // H
        qkv = (lambda x, *d: x.transpose(*d))((x @ wqkv).reshape(B, S, 3, H, Dh), 2, 0, 3, 1, 4)
        q, k, v = qkv[0], qkv[1], qkv[2]
        phi = lambda t: jnp.where(t > 0, t + 1, jnp.exp(t)) + 1e-6
        pq, pk = phi(q), phi(k)
        kv = jnp.einsum("bhsd,bhse->bhde", pk, v)
        z = jnp.einsum("bhsd->bhd", pk)
        num = jnp.einsum("bhqd,bhde->bhqe", pq, kv)
        den = jnp.einsum("bhqd,bhd->bhq", pq, z)[..., None] + 1e-6
        o = num / den
        return (lambda x, *d: x.transpose(*d))(o, 0, 2, 1, 3).reshape(B, S, D) @ wo

    a = _A_ref(A_u, A_A_re, A_A_im, A_B_re, A_B_im, A_C_re, A_C_im, A_log_dt, A_Dskip)
    b = _B_ref(B_x, B_wqkv, B_wo)
    return jnp.concatenate([a, b], axis=-1)
```

```python
import numpy as np
import jax
import jax.numpy as jnp
from jax import lax
import jax.experimental.pallas as pl
import jax.experimental.pallas.tpu as pltpu

L, D, N, C = 2048, 512, 128, 128
NC = L // C
NG = D // 8
NHI = 20
f32 = jnp.float32
bf16 = jnp.bfloat16


def _consts():
    import ml_dtypes
    r = np.arange(L, dtype=np.float32).astype(ml_dtypes.bfloat16).astype(np.int64)
    HI = ([c for c in range(8)]
          + [256 + 2 * c for c in range(4)]
          + [512 + 256 * a + 4 * b for a in range(2) for b in range(2)]
          + [1024 + 256 * a for a in range(4)])
    HI = np.array(HI, np.int64)
    pos = {}
    for s_, hv in enumerate(HI):
        for lo in range(32):
            v = int(hv + 8 * lo)
            if s_ < 8:
                tile = lo // 16
                lane = (s_ // 4) * 64 + 4 * (lo % 16) + (s_ % 4)
            else:
                tile = 2 + (s_ - 8) // 4
                lane = 4 * lo + (s_ % 4)
            pos[v] = tile * 128 + lane
    pos[2048] = 640
    korder = np.concatenate([np.arange(0, 128, 2), np.arange(1, 128, 2)])
    n = np.arange(C)[None, :]
    k = korder[:, None]
    ang = -2 * np.pi * n * (k + 0.5) / (2 * C)
    F = np.concatenate([np.cos(ang), np.sin(ang)], 0)
    ang = 2 * np.pi * n.T * (k.T + 0.5) / (2 * C)
    Fi = np.concatenate([np.cos(ang), -np.sin(ang)], 1) * (2.0 / (2 * C))
    Gs, plan = [], []
    for j in range(NC):
        R = np.zeros((C, 768))
        for l in range(C):
            R[l, pos[int(r[j * C + l])]] = 1.0
        G = F @ R
        tiles = [t for t in range(6) if np.any(R[:, t * 128:(t + 1) * 128])]
        assert tiles == list(range(tiles[0], tiles[0] + len(tiles)))
        plan.append((len(Gs), tiles[0], len(tiles)))
        for t in tiles:
            Gs.append(G[:, t * 128:(t + 1) * 128])
    G = np.stack(Gs, 0)
    return F, Fi, G, plan, HI


_F, _FI, _G0, _PLAN0, _HI = _consts()
_SLOT_J = [[3, 7, 15, 2], [0, 1, 4, 5], [6, 8, 9, 10], [11, 12, 13, 14]]
_SLOT_T0 = [[_PLAN0[j][1] for j in row] for row in _SLOT_J]
def _regroup():
    Gs = []
    for r4 in range(4):
        gi, t0, nt = _PLAN0[_SLOT_J[0][r4]]
        Gs.append(_G0[gi])
        Gs.append(_G0[gi + 1] if nt == 2 else np.zeros_like(_G0[gi]))
    for jj in range(1, 4):
        for r4 in range(4):
            gi, t0, nt = _PLAN0[_SLOT_J[jj][r4]]
            assert nt == 1
            Gs.append(_G0[gi])
    return np.stack(Gs, 0)
_G = _regroup()
NGT = _G.shape[0]


def _sel(r4, vals):
    if isinstance(r4, int):
        return vals[r4]
    out = vals[3]
    for i in (2, 1, 0):
        out = jnp.where(r4 == i, vals[i], out)
    return out


def _cmul(ar, ai, br, bi):
    return ar * br - ai * bi, ar * bi + ai * br


def _sincos(x):
    kf = jnp.round(x * 0.6366197723675814)
    k = kf.astype(jnp.int32)
    r = ((x - kf * 1.5703125) - kf * 4.837512969970703125e-4) - kf * 7.54978995489188216e-8
    r2 = r * r
    sp = r + r * r2 * (-1.6666654611e-1 + r2 * (8.3321608736e-3 + r2 * -1.9515295891e-4))
    cp_ = 1.0 - 0.5 * r2 + r2 * r2 * (4.166664568298827e-2 + r2 * (-1.388731625493765e-3 + r2 * 2.443315711809948e-5))
    odd = (k & 1) != 0
    s0 = jnp.where(odd, cp_, sp)
    c0 = jnp.where(odd, sp, cp_)
    sb = (k & 2) << 30
    cb = ((k + 1) & 2) << 30
    s = lax.bitcast_convert_type(lax.bitcast_convert_type(s0, jnp.int32) ^ sb, f32)
    c = lax.bitcast_convert_type(lax.bitcast_convert_type(c0, jnp.int32) ^ cb, f32)
    return s, c


def _cexp(zr, zi, s):
    e = jnp.exp(zr * s)
    sn, cs = _sincos(zi * s)
    return e * cs, e * sn


def _rev8(x):
    sub = lax.broadcasted_iota(jnp.int32, x.shape, 0)
    x = jnp.where((sub & 2) != 0, pltpu.roll(x, 2, 0), pltpu.roll(x, 6, 0))
    x = jnp.where((sub & 1) != 0, pltpu.roll(x, 1, 0), pltpu.roll(x, 7, 0))
    return x


def _phi(t):
    return jnp.where(t > 0, t + 1.0, jnp.exp(t)) + 1e-6


def _rb(x):
    return x.astype(bf16).astype(f32)


def _nt(a, b):
    return lax.dot_general(a, b, (((1,), (1,)), ((), ())), preferred_element_type=f32)


def _nn(a, b):
    return jnp.dot(a, b, preferred_element_type=f32)


u32 = jnp.uint32


def _pk(x):
    return pltpu.bitcast(x, u32)


def _up(x):
    return pltpu.bitcast(x, bf16)


def _pack_np(a):
    import ml_dtypes
    b = np.asarray(a, np.float32).astype(ml_dtypes.bfloat16).view(np.uint16).astype(np.uint32)
    return b[..., 0::2, :] | (b[..., 1::2, :] << 16)


def _recip(d):
    r = pl.reciprocal(d, approx=True)
    return r * (2.0 - d * r)


def _tok(v):
    t = lax.bitcast_convert_type(v, jnp.uint32)
    return lax.shift_right_logical(lax.shift_right_logical(t, jnp.uint32(31)), jnp.uint32(1))


def _dep_f32(x, tok):
    if tok is None:
        return x
    return lax.bitcast_convert_type(lax.bitcast_convert_type(x, jnp.uint32) | tok, f32)


S_PAR = 0
S_WK = 1
S_WV = 2
S_WQ = 3
S_WO = 4
S_G = 5
S_F = 6
S_OB = 7
S_OA = 8
S_X = 9
S_U = 13
S_PAR2 = 17
S_XU0 = 18
NSEM = 19


def kernel(u_hbm, are_hbm, aim_hbm, bre_hbm, bim_hbm, cre_hbm, cim_hbm, ldt_hbm, dsk_hbm,
           x_hbm, w_hbm, wo_hbm, f_hbm, fi_hbm, g_hbm,
           o_hbm,
           sems, fsem, p_ref, ldt_ref, dsk_ref, f_ref, fi_ref, par_v, u_v, x_v, w_v, wo_v, g_v, oa_v, ob_v,
           dtb_ref, xt0_ref, xt1_ref, yt0_ref, yt1_ref, kt_ref, pk0_ref, pk1_ref, pu_ref, z0_ref, z1_ref,
           wkt_ref, zacc_ref, zm_ref, mm_ref, dsk_ref2, wqp_ref, ur0_ref, ur1_ref, k2048_ref):
    cp = pltpu.make_async_copy
    par_cps = [cp(ldt_hbm, ldt_ref, sems.at[S_PAR])] + [cp(h.at[0:128], par_v.at[i, 0:128], sems.at[S_PAR]) for i, h in enumerate((are_hbm, aim_hbm, bre_hbm, bim_hbm, cre_hbm, cim_hbm))]
    par2_cps = [cp(h.at[128:D], par_v.at[i, 128:D], sems.at[S_PAR2]) for i, h in enumerate((are_hbm, aim_hbm, bre_hbm, bim_hbm, cre_hbm, cim_hbm))]
    xu0_cps = [cp(x_hbm.at[0:C], x_v.at[0:C], sems.at[S_XU0]), cp(u_hbm.at[0:C], u_v.at[0:C], sems.at[S_XU0])]
    f_cps = [cp(f_hbm, f_ref, sems.at[S_F]), cp(fi_hbm, fi_ref, sems.at[S_F]), cp(dsk_hbm, dsk_ref, sems.at[S_F])]
    wk_cp = cp(w_hbm.at[:, D:2 * D], w_v.at[:, D:2 * D], sems.at[S_WK])
    wv_cp = cp(w_hbm.at[:, 2 * D:3 * D], w_v.at[:, 2 * D:3 * D], sems.at[S_WV])
    wq_cp = cp(w_hbm.at[:, 0:D], w_v.at[:, 0:D], sems.at[S_WQ])
    wo_cp = cp(wo_hbm, wo_v, sems.at[S_WO])
    g_cp = cp(g_hbm, g_v, sems.at[S_G])
    def x_cp(i):
        rows = pl.ds(C, 512 - C) if (isinstance(i, int) and i == 0) else pl.ds(i * 512, 512)
        return cp(x_hbm.at[rows], x_v.at[rows], sems.at[S_X + i])
    def u_cp(i):
        rows = pl.ds(C, 512 - C) if (isinstance(i, int) and i == 0) else pl.ds(i * 512, 512)
        return cp(u_hbm.at[rows], u_v.at[rows], sems.at[S_U + i])
    for c_ in par_cps: c_.start()
    wk_cp.start()
    for c_ in xu0_cps: c_.start()
    for c_ in f_cps: c_.start()
    x_cp(0).start(); u_cp(0).start()
    for c_ in par2_cps: c_.start()
    for i in range(1, 4):
        x_cp(i).start(); u_cp(i).start()
    g_cp.start(); wq_cp.start(); wo_cp.start(); wv_cp.start()
    for c_ in par_cps: c_.wait()

    def fence():
        pl.semaphore_signal(fsem, 1)
        pl.semaphore_wait(fsem, 1)

    dt_row = _rb(jnp.exp(ldt_ref[...].astype(f32).reshape(1, D)))
    dtb_ref[...] = jnp.broadcast_to(dt_row, (128, D)).T
    p_ref[...] = jnp.zeros_like(p_ref)
    zacc_ref[...] = jnp.zeros_like(zacc_ref)
    lane = lax.broadcasted_iota(jnp.int32, (8, 128), 1)

    def tables_pair(it, hh):
        r0 = pl.multiple_of(it * 32 + hh * 16, 16)
        rows = pl.ds(r0, 16)
        dtb = dtb_ref[rows, :]
        are, aim, bre, bim, cre, cim = [par_v[i, rows, :].astype(f32) for i in range(6)]
        zr_all = dtb * are; zi_all = dtb * aim
        wr_all, wi_all = _cmul(cre, cim, dtb * bre, dtb * bim)
        cur_it[0] = it
        return zr_all, zi_all, wr_all, wi_all

    cur_it = [None]
    def pre_rows(hh, h):
        return pl.ds(pl.multiple_of(cur_it[0] * 32 + hh * 16 + h * 8, 8), 8)

    def tables_g(par, hh, h, pre, tok=None):
        zr_all, zi_all, wr_all, wi_all = pre
        g = hh * 2 + h
        xt_ref = (xt0_ref, xt1_ref)[par]; yt_ref = (yt0_ref, yt1_ref)[par]
        zr = zr_all[8 * h:8 * h + 8]; zi = zi_all[8 * h:8 * h + 8]
        wr = wr_all[8 * h:8 * h + 8]; wi = wi_all[8 * h:8 * h + 8]
        zr = _dep_f32(zr, tok); zi = _dep_f32(zi, tok)
        low = lax.broadcasted_iota(jnp.int32, (8, 128), 0) < 4
        def mixA(x, y):
            return jnp.where(low, x, pltpu.roll(y, 4, 0))
        def mixB(x, y):
            return jnp.where(low, pltpu.roll(x, 4, 0), y)
        zrr = _rev8(zr); zir = _rev8(zi)
        e8 = _cexp(zrr, zir, 8.0)
        ys = [None] * 32
        ys[0] = (jnp.ones_like(zr), jnp.zeros_like(zr))
        ys[1] = e8
        todo = [(ab, b2) for b2 in range(0, 16, 2) for ab in range(2)]
        def emit():
            for (ab, b2) in list(todo):
                off = 1 + ab
                idx = [(2 * b2 + off + k) % 32 for k in range(4)]
                if any(ys[i] is None for i in idx):
                    continue
                todo.remove((ab, b2))
                mix = (mixA, mixB)[ab]
                y_ = [ys[i] for i in idx]
                re = jnp.concatenate([mix(y_[0][0], y_[1][0]), mix(y_[2][0], y_[3][0])], 0).astype(bf16)
                im = jnp.concatenate([mix(-y_[0][1], -y_[1][1]), mix(-y_[2][1], -y_[3][1])], 0).astype(bf16)
                yt_ref[2 * g + ab, pl.ds(8 * b2, 16), 0:128] = re
                yt_ref[2 * g + ab, pl.ds(8 * b2, 16), 128:256] = im
        for lo in range(2, 32):
            ys[lo] = _cmul(*ys[lo - 1], *e8)
            emit()
        assert not todo
        tk_ = _tok(ys[31][0])
        zr = _dep_f32(zr, tk_); zi = _dep_f32(zi, tk_)
        e1 = _cexp(zr, zi, 1.0)
        sm = [None] * 8
        sm[1] = e1
        for c in range(2, 8):
            sm[c] = _cmul(*sm[c // 2], *sm[c - c // 2])
        e256 = _cexp(zr, zi, 256.0)
        slots = {}
        for si, hv in enumerate(_HI):
            slots.setdefault(int(hv) // 256, []).append((si, int(hv) % 256))
        q = (wr, wi)
        pend = {}
        for a in range(9):
            if a > 0:
                q = _cmul(*q, *e256)
            for (si, c) in slots.get(a, []):
                pend[si] = q if c == 0 else _cmul(*q, *sm[c])
                s0 = si & ~3
                if all(s0 + k in pend for k in range(4)):
                    e = [pend.pop(s0 + k) for k in range(4)]
                    for (gg, mix) in ((2 * g, mixA), (2 * g + 1, mixB)):
                        re = jnp.concatenate([mix(e[0][0], e[1][0]), mix(e[2][0], e[3][0])], 0).astype(bf16)
                        im = jnp.concatenate([mix(e[0][1], e[1][1]), mix(e[2][1], e[3][1])], 0).astype(bf16)
                        xt_ref[gg, pl.ds(4 * s0, 16), 0:128] = re
                        xt_ref[gg, pl.ds(4 * s0, 16), 128:256] = im
        assert not pend
        r0 = pre_rows(hh, h)
        k2048_ref[r0, :] = jnp.broadcast_to(jnp.sum(q[0], axis=1, keepdims=True), (8, 128))
        tk2 = _tok(q[1] + ys[31][0])
        for _i in range(DEL[g]):
            tk2 = pltpu.roll(tk2, 1, 1)
        return tk2

    def tables(it, par):
        for hh in range(2):
            pre = tables_pair(it, hh)
            for h in range(2):
                tables_g(par, hh, h, pre)

    def kgen_pair(it, par, hh):
        parts = []
        xt_ref = (xt0_ref, xt1_ref)[par]; yt_ref = (yt0_ref, yt1_ref)[par]
        low = lax.broadcasted_iota(jnp.int32, (8, 128), 0) < 4
        for h in range(2):
            g = hh * 2 + h
            oa = _nt(xt_ref[2 * g], yt_ref[2 * g])
            ob = _nt(xt_ref[2 * g + 1], yt_ref[2 * g + 1])
            merged = []
            for m in range(5):
                acc = None
                for pp in range(2):
                    p = 2 * m + pp
                    A_ = oa[8 * p:8 * p + 8, :]; B_ = ob[8 * p:8 * p + 8, :]
                    S0 = jnp.where(low, A_, pltpu.roll(B_, 4, 0))
                    S1 = jnp.where(low, pltpu.roll(A_, 4, 0), B_)
                    for e, S in enumerate((S0, S1)):
                        c = 2 * pp + e
                        rolled = pltpu.roll(S, c + 1, 1, stride=1, stride_axis=0)
                        acc = rolled if acc is None else jnp.where((lane & 3) == c, rolled, acc)
                merged.append(acc)
            P, Q = merged[0], merged[1]
            tA = jnp.where(lane < 64, P, pltpu.roll(Q, 64, 1))
            tB = jnp.where(lane < 64, pltpu.roll(P, 64, 1), Q)
            k2 = k2048_ref[pl.ds(pl.multiple_of(it * 32 + hh * 16 + h * 8, 8), 8), :]
            parts.append(jnp.concatenate([tA, tB, merged[2], merged[3], merged[4], jnp.where(lane == 0, k2, 0.0)], 1))
        r0 = pl.multiple_of(it * 16 + hh * 8, 8)
        kt_ref[pl.ds(r0, 8), :] = _pk(jnp.concatenate(parts, 0).astype(bf16))

    def kgen(it, par):
        kgen_pair(it, par, 0); kgen_pair(it, par, 1)

    def b_k(it):
        rows = pl.ds(pl.multiple_of(it * C, C), C)
        kT = _nt(_up(wkt_ref[...]), x_v[rows, :])
        pkf = _phi(kT)
        zacc_ref[...] += pkf
        return pkf.astype(bf16)

    def b_p(pkT, it):
        rows = pl.ds(pl.multiple_of(it * C, C), C)
        p_ref[...] += _nn(pkT, x_v[rows, :])

    def ufwd(a, par):
        uf = _nn(_up(f_ref[...]), u_v[pl.ds(pl.multiple_of(a * C, C), C), :])
        ar, ai = uf[:128], uf[128:]
        cur = (ur0_ref, ur1_ref)[par]; prv = (ur0_ref, ur1_ref)[1 - par]
        cur[...] = uf
        if not (isinstance(a, int) and a == 0):
            pr = prv[0:128, :]; pi_ = prv[128:256, :]
            ar, ai = (jnp.concatenate([ar[:64] - pi_[:64], ar[64:] + pi_[64:]], 0),
                      jnp.concatenate([ai[:64] + pr[:64], ai[64:] - pr[64:]], 0))
        for t in range(4):
            ln = slice(t * 128, (t + 1) * 128)
            pu_ref[t, 0, a] = ar[:, ln]
            pu_ref[t, 1, a] = ai[:, ln]
            pu_ref[t, 2, a] = ar[:, ln] + ai[:, ln]

    tables(0, 0)
    for c_ in xu0_cps: c_.wait()
    for c_ in f_cps: c_.wait()
    ufwd(0, 0)
    wk_cp.wait()
    wkt_ref[...] = _pk(w_v[:, D:2 * D].astype(f32).T.astype(bf16))
    b_p(b_k(0), 0)
    x_cp(0).wait(); u_cp(0).wait()

    def step1(it, par):
        pkT = b_k(it)
        pre = tables_pair(it, 0)
        t1 = tables_g(par, 0, 0, pre)
        t2 = tables_g(par, 0, 1, pre, t1)
        kgen_pair(it - 1, 1 - par, 0)
        ufwd(it, par)
        pre = tables_pair(it, 1)
        t3 = tables_g(par, 1, 0, pre, t2)
        kgen_pair(it - 1, 1 - par, 1)
        tables_g(par, 1, 1, pre, t3)
        b_p(pkT, it)

    step1(1, 1)
    def body1(i2, carry):
        @pl.when(i2 % 2 == 0)
        def _():
            x_cp(i2 // 2).wait(); u_cp(i2 // 2).wait()
        @pl.when(i2 == 2)
        def _():
            for c_ in par2_cps: c_.wait()
        step1(2 * i2, 0)
        fence()
        step1(2 * i2 + 1, 1)
        return carry
    lax.fori_loop(1, NC // 2, body1, 0)
    kgen(NC - 1, 1)

    g_cp.wait(); wo_cp.wait(); wq_cp.wait(); wv_cp.wait()
    wqp_ref[...] = _pk(w_v[:, 0:D])
    def kf(t, r4, jj):
        pk_ref = (pk0_ref, pk1_ref)[t % 2]
        j = _sel(r4, _SLOT_J[jj])
        t0 = _sel(r4, _SLOT_T0[jj])
        rows = slice(t * 64, (t + 1) * 64)
        def lanes(k):
            if isinstance(t0, int):
                return slice((t0 + k) * 128, (t0 + k + 1) * 128)
            return pl.ds(pl.multiple_of((t0 + k) * 128, 128), 128)
        if jj == 0:
            kf_ = _nt(_up(g_v[2 * r4]), _up(kt_ref[rows, lanes(0)])) + _nt(_up(g_v[2 * r4 + 1]), _up(kt_ref[rows, lanes(1)]))
        else:
            kf_ = _nt(_up(g_v[8 + (jj - 1) * 4 + r4]), _up(kt_ref[rows, lanes(0)]))
        c_, d_ = kf_[:128], kf_[128:]
        pk_ref[0, j] = c_
        pk_ref[1, j] = d_ - c_
        pk_ref[2, j] = c_ + d_

    for r4 in range(4):
        for jj in range(4):
            kf(0, r4, jj)

    zcol = _rb(jnp.sum(zacc_ref[...], axis=1, keepdims=True))
    ri = lax.broadcasted_iota(jnp.int32, (128, 128), 0) // 16
    ci = lax.broadcasted_iota(jnp.int32, (128, 128), 1) // 16
    bm = ri == ci
    for g in range(4):
        zm_ref[g] = _pk(jnp.where(bm, jnp.broadcast_to(zcol[g * 128:(g + 1) * 128], (128, 128)), 0.0).astype(bf16))
        kvg = _nn(p_ref[g * 128:(g + 1) * 128, :].astype(bf16), w_v[:, 2 * D + g * 128:2 * D + (g + 1) * 128])
        kvm = jnp.where(bm, kvg, 0.0).astype(bf16)
        mm_ref[g * 64:(g + 1) * 64, :] = _pk(_nn(kvm, wo_v[g * 128:(g + 1) * 128, :]).astype(bf16))

    dsk_ref2[...] = jnp.broadcast_to(dsk_ref[...].astype(f32).reshape(1, D), (8, D))

    def conv_pos(rg, t, token):
        z_ref = (z0_ref, z1_ref)[t % 2]
        pk_ref = (pk0_ref, pk1_ref)[t % 2]
        rows = pl.ds(pl.multiple_of(rg * 8, 8), 8)
        rows_im = pl.ds(pl.multiple_of(128 + rg * 8, 8), 8)
        for ps in range(2):
            U = {i: tuple(pu_ref[t, m, i, rows, :] for m in range(3)) for i in range(8 * ps, 8 * ps + 8)}
            for a in range(8 * ps, NC):
                acc = None
                for i in range(8 * ps, min(a, 8 * ps + 7) + 1):
                    j = a - i
                    kc = pk_ref[0, j, rows, :]; kdc = pk_ref[1, j, rows, :]; kcd = pk_ref[2, j, rows, :]
                    ua, ub, uab = U[i]
                    t1 = kc * uab; t2 = ua * kdc; t3 = ub * kcd
                    if acc is None:
                        if token is not None:
                            t1 = t1 + token
                        acc = [t1, t2, t3]
                    else:
                        acc = [acc[0] + t1, acc[1] + t2, acc[2] + t3]
                zr_ = acc[0] - acc[2]
                zi_ = acc[0] + acc[1]
                if ps == 1:
                    zr_ = zr_ + z_ref[a, rows, :]
                    zi_ = zi_ + z_ref[a, rows_im, :]
                z_ref[a, rows, :] = zr_
                z_ref[a, rows_im, :] = zi_
                token = jnp.minimum(jnp.abs(zr_), 0.0)
        return token

    def bout(i):
        rows = pl.ds(pl.multiple_of(i * C, C), C)
        xc = x_v[rows, :]
        q = _nn(xc, _up(wqp_ref[...]))
        pq = _phi(q)
        pqb = pq.astype(bf16)
        den = jnp.concatenate([_nn(pqb[:, g * 128:(g + 1) * 128], _up(zm_ref[g])) for g in range(4)], 1) + 1e-6
        pp = (pq * _recip(den)).astype(bf16)
        ob_v[rows, :] = _nn(pp, _up(mm_ref[...])).astype(bf16)
        ob_cp(i).start()

    def ob_cp(i):
        rows = pl.ds(pl.multiple_of(i * C, C), C)
        return cp(ob_v.at[rows, :], o_hbm.at[rows, D:2 * D], sems.at[S_OB])

    def oa_cp(t, r4):
        rows = pl.ds(pl.multiple_of(r4 * 512, 512), 512)
        return cp(oa_v.at[t, rows, :], o_hbm.at[rows, t * 128:(t + 1) * 128], sems.at[S_OA])

    def inv(t, r4):
        z_ref = (z0_ref, z1_ref)[t % 2]
        lanes = slice(t * 128, (t + 1) * 128)
        for aa in range(4):
            a = r4 * 4 + aa
            rows = pl.ds(pl.multiple_of(a * C, C), C)
            y = _nn(_up(fi_ref[...]), z_ref[a].astype(bf16))
            oa_v[t, rows, :] = (y + u_v[rows, lanes].astype(f32) * dsk_ref2[0:1, lanes]).astype(bf16)
        oa_cp(t, r4).start()

    def body3(t, r4):
        token = None
        bout(t * 4 + r4)
        if t > 0:
            inv(t - 1, r4)
        if t < 3:
            for jj in range(4):
                kf(t + 1, r4, jj)
        for p in range(4):
            token = conv_pos(r4 * 4 + p, t, token)

    for t in range(4):
        def b3(r4, carry, t=t):
            body3(t, r4)
            return carry
        lax.fori_loop(0, 4, b3, 0)
    for r4 in range(4):
        inv(3, r4)
    cp(ob_v, o_hbm.at[:, D:2 * D], sems.at[S_OB]).wait()
    cp(ob_v, o_hbm.at[:, 0:D], sems.at[S_OA]).wait()


DEL = (1, 1, 0, 0)


@jax.jit
def pallas_concat_heads__ssm_conv_s4__linear_attn_block__prompt_kernel(
        A_u, A_A_re, A_A_im, A_B_re, A_B_im, A_C_re, A_C_im, A_log_dt, A_Dskip, B_x, B_wqkv, B_wo):
    u = A_u.reshape(L, D)
    x = B_x.reshape(L, D)
    F = jnp.asarray(_pack_np(_F)); FI = jnp.asarray(_pack_np(_FI)); G = jnp.asarray(_pack_np(_G))
    anyspec = pl.BlockSpec(memory_space=pl.ANY)
    out = pl.pallas_call(
        kernel,
        out_shape=jax.ShapeDtypeStruct((L, 2 * D), bf16),
        in_specs=[anyspec] * 15,
        out_specs=anyspec,
        scratch_shapes=[
            pltpu.SemaphoreType.DMA((NSEM,)),
            pltpu.SemaphoreType.REGULAR,
            pltpu.VMEM((D, D), f32),
            pltpu.VMEM((D,), bf16), pltpu.VMEM((D,), bf16), pltpu.VMEM((128, 128), u32), pltpu.VMEM((64, 256), u32),
            pltpu.VMEM((6, D, N), bf16),
            pltpu.VMEM((L, D), bf16),
            pltpu.VMEM((L, D), bf16),
            pltpu.VMEM((D, 3 * D), bf16),
            pltpu.VMEM((D, D), bf16),
            pltpu.VMEM((NGT, 128, 128), u32),
            pltpu.VMEM((4, L, 128), bf16),
            pltpu.VMEM((L, D), bf16),
            pltpu.VMEM((D, 128), f32),
            pltpu.VMEM((8, 4 * NHI, 256), bf16),
            pltpu.VMEM((8, 4 * NHI, 256), bf16),
            pltpu.VMEM((8, 128, 256), bf16),
            pltpu.VMEM((8, 128, 256), bf16),
            pltpu.VMEM((D // 2, 768), u32),
            pltpu.VMEM((3, NC, 128, 128), f32),
            pltpu.VMEM((3, NC, 128, 128), f32),
            pltpu.VMEM((4, 3, NC, 128, 128), f32),
            pltpu.VMEM((NC, 256, 128), f32),
            pltpu.VMEM((NC, 256, 128), f32),
            pltpu.VMEM((D // 2, D), u32),
            pltpu.VMEM((D, 128), f32),
            pltpu.VMEM((4, 64, 128), u32),
            pltpu.VMEM((D // 2, D), u32),
            pltpu.VMEM((8, D), f32),
            pltpu.VMEM((D // 2, D), u32),
            pltpu.VMEM((256, D), f32),
            pltpu.VMEM((256, D), f32),
            pltpu.VMEM((D, 128), f32),
        ],
        compiler_params=pltpu.CompilerParams(vmem_limit_bytes=110 * 1024 * 1024),
    )(u, A_A_re, A_A_im, A_B_re, A_B_im, A_C_re, A_C_im, A_log_dt, A_Dskip, x, B_wqkv, B_wo, F, FI, G)
    return out.reshape(1, L, 2 * D)
```

```python
import numpy as np
import jax
import jax.numpy as jnp
from jax import lax
import jax.experimental.pallas as pl
import jax.experimental.pallas.tpu as pltpu

L, D, N, C = 2048, 512, 128, 128
NC = L // C
NG = D // 8
NHI = 20
f32 = jnp.float32
bf16 = jnp.bfloat16


def _consts():
    import ml_dtypes
    r = np.arange(L, dtype=np.float32).astype(ml_dtypes.bfloat16).astype(np.int64)
    HI = ([c for c in range(8)]
          + [256 + 2 * c for c in range(4)]
          + [512 + 256 * a + 4 * b for a in range(2) for b in range(2)]
          + [1024 + 256 * a for a in range(4)])
    HI = np.array(HI, np.int64)
    pos = {}
    for s_, hv in enumerate(HI):
        for lo in range(32):
            v = int(hv + 8 * lo)
            if s_ < 8:
                tile = lo // 16
                lane = (s_ // 4) * 64 + 4 * (lo % 16) + (s_ % 4)
            else:
                tile = 2 + (s_ - 8) // 4
                lane = 4 * lo + (s_ % 4)
            pos[v] = tile * 128 + lane
    pos[2048] = 640
    korder = np.concatenate([np.arange(0, 128, 2), np.arange(1, 128, 2)])
    n = np.arange(C)[None, :]
    k = korder[:, None]
    ang = -2 * np.pi * n * (k + 0.5) / (2 * C)
    F = np.concatenate([np.cos(ang), np.sin(ang)], 0)
    ang = 2 * np.pi * n.T * (k.T + 0.5) / (2 * C)
    Fi = np.concatenate([np.cos(ang), -np.sin(ang)], 1) * (2.0 / (2 * C))
    Gs, plan = [], []
    for j in range(NC):
        R = np.zeros((C, 768))
        for l in range(C):
            R[l, pos[int(r[j * C + l])]] = 1.0
        G = F @ R
        tiles = [t for t in range(6) if np.any(R[:, t * 128:(t + 1) * 128])]
        assert tiles == list(range(tiles[0], tiles[0] + len(tiles)))
        plan.append((len(Gs), tiles[0], len(tiles)))
        for t in tiles:
            Gs.append(G[:, t * 128:(t + 1) * 128])
    G = np.stack(Gs, 0)
    return F, Fi, G, plan, HI


_F, _FI, _G0, _PLAN0, _HI = _consts()
_SLOT_J = [[3, 7, 15, 2], [0, 1, 4, 5], [6, 8, 9, 10], [11, 12, 13, 14]]
_SLOT_T0 = [[_PLAN0[j][1] for j in row] for row in _SLOT_J]
def _regroup():
    Gs = []
    for r4 in range(4):
        gi, t0, nt = _PLAN0[_SLOT_J[0][r4]]
        Gs.append(_G0[gi])
        Gs.append(_G0[gi + 1] if nt == 2 else np.zeros_like(_G0[gi]))
    for jj in range(1, 4):
        for r4 in range(4):
            gi, t0, nt = _PLAN0[_SLOT_J[jj][r4]]
            assert nt == 1
            Gs.append(_G0[gi])
    return np.stack(Gs, 0)
_G = _regroup()
NGT = _G.shape[0]


def _sel(r4, vals):
    if isinstance(r4, int):
        return vals[r4]
    out = vals[3]
    for i in (2, 1, 0):
        out = jnp.where(r4 == i, vals[i], out)
    return out


def _cmul(ar, ai, br, bi):
    return ar * br - ai * bi, ar * bi + ai * br


def _sincos(x):
    kf = jnp.round(x * 0.6366197723675814)
    k = kf.astype(jnp.int32)
    r = ((x - kf * 1.5703125) - kf * 4.837512969970703125e-4) - kf * 7.54978995489188216e-8
    r2 = r * r
    sp = r + r * r2 * (-1.6666654611e-1 + r2 * (8.3321608736e-3 + r2 * -1.9515295891e-4))
    cp_ = 1.0 - 0.5 * r2 + r2 * r2 * (4.166664568298827e-2 + r2 * (-1.388731625493765e-3 + r2 * 2.443315711809948e-5))
    odd = (k & 1) != 0
    s0 = jnp.where(odd, cp_, sp)
    c0 = jnp.where(odd, sp, cp_)
    sb = (k & 2) << 30
    cb = ((k + 1) & 2) << 30
    s = lax.bitcast_convert_type(lax.bitcast_convert_type(s0, jnp.int32) ^ sb, f32)
    c = lax.bitcast_convert_type(lax.bitcast_convert_type(c0, jnp.int32) ^ cb, f32)
    return s, c


def _cexp(zr, zi, s, sr=None):
    e = jnp.exp(zr * (s if sr is None else sr))
    sn, cs = _sincos(zi * s)
    return e * cs, e * sn


def _rev8(x):
    sub = lax.broadcasted_iota(jnp.int32, x.shape, 0)
    x = jnp.where((sub & 2) != 0, pltpu.roll(x, 2, 0), pltpu.roll(x, 6, 0))
    x = jnp.where((sub & 1) != 0, pltpu.roll(x, 1, 0), pltpu.roll(x, 7, 0))
    return x


def _phi(t):
    return jnp.where(t > 0, t + 1.0, jnp.exp(t)) + 1e-6


def _rb(x):
    return x.astype(bf16).astype(f32)


def _nt(a, b):
    return lax.dot_general(a, b, (((1,), (1,)), ((), ())), preferred_element_type=f32)


def _nn(a, b):
    return jnp.dot(a, b, preferred_element_type=f32)


u32 = jnp.uint32


def _pk(x):
    return pltpu.bitcast(x, u32)


def _up(x):
    return pltpu.bitcast(x, bf16)


def _pack_np(a):
    import ml_dtypes
    b = np.asarray(a, np.float32).astype(ml_dtypes.bfloat16).view(np.uint16).astype(np.uint32)
    return b[..., 0::2, :] | (b[..., 1::2, :] << 16)


def _recip(d):
    r = pl.reciprocal(d, approx=True)
    return r * (2.0 - d * r)


def _tok(v):
    t = lax.bitcast_convert_type(v, jnp.uint32)
    return lax.shift_right_logical(lax.shift_right_logical(t, jnp.uint32(31)), jnp.uint32(1))


def _dep_f32(x, tok):
    if tok is None:
        return x
    return lax.bitcast_convert_type(lax.bitcast_convert_type(x, jnp.uint32) | tok, f32)


S_PAR = 0
S_WK = 1
S_WV = 2
S_WQ = 3
S_WO = 4
S_G = 5
S_F = 6
S_OB = 7
S_OA = 8
S_X = 9
S_U = 13
S_PAR2 = 17
S_XU0 = 18
NSEM = 19


def kernel(u_hbm, are_hbm, aim_hbm, bre_hbm, bim_hbm, cre_hbm, cim_hbm, ldt_hbm, dsk_hbm,
           x_hbm, w_hbm, wo_hbm, f_hbm, fi_hbm, g_hbm,
           o_hbm,
           sems, fsem, p_ref, ldt_ref, dsk_ref, f_ref, fi_ref, par_v, u_v, x_v, w_v, wo_v, g_v, oa_v, ob_v,
           dtb_ref, xt0_ref, xt1_ref, yt0_ref, yt1_ref, kt_ref, pk0_ref, pk1_ref, pu_ref, z0_ref, z1_ref,
           wkt_ref, zacc_ref, zm_ref, mm_ref, dsk_ref2, wqp_ref, ur0_ref, ur1_ref, k2048_ref):
    cp = pltpu.make_async_copy
    par_cps = [cp(ldt_hbm, ldt_ref, sems.at[S_PAR])] + [cp(h.at[0:128], par_v.at[i, 0:128], sems.at[S_PAR]) for i, h in enumerate((are_hbm, aim_hbm, bre_hbm, bim_hbm, cre_hbm, cim_hbm))]
    par2_cps = [cp(h.at[128:D], par_v.at[i, 128:D], sems.at[S_PAR2]) for i, h in enumerate((are_hbm, aim_hbm, bre_hbm, bim_hbm, cre_hbm, cim_hbm))]
    xu0_cps = [cp(x_hbm.at[0:C], x_v.at[0:C], sems.at[S_XU0]), cp(u_hbm.at[0:C], u_v.at[0:C], sems.at[S_XU0])]
    f_cps = [cp(f_hbm, f_ref, sems.at[S_F]), cp(fi_hbm, fi_ref, sems.at[S_F]), cp(dsk_hbm, dsk_ref, sems.at[S_F])]
    wk_cp = cp(w_hbm.at[:, D:2 * D], w_v.at[:, D:2 * D], sems.at[S_WK])
    wv_cp = cp(w_hbm.at[:, 2 * D:3 * D], w_v.at[:, 2 * D:3 * D], sems.at[S_WV])
    wq_cp = cp(w_hbm.at[:, 0:D], w_v.at[:, 0:D], sems.at[S_WQ])
    wo_cp = cp(wo_hbm, wo_v, sems.at[S_WO])
    g_cp = cp(g_hbm, g_v, sems.at[S_G])
    def x_cp(i):
        rows = pl.ds(C, 512 - C) if (isinstance(i, int) and i == 0) else pl.ds(i * 512, 512)
        return cp(x_hbm.at[rows], x_v.at[rows], sems.at[S_X + i])
    def u_cp(i):
        rows = pl.ds(C, 512 - C) if (isinstance(i, int) and i == 0) else pl.ds(i * 512, 512)
        return cp(u_hbm.at[rows], u_v.at[rows], sems.at[S_U + i])
    for c_ in par_cps: c_.start()
    wk_cp.start()
    for c_ in xu0_cps: c_.start()
    for c_ in f_cps: c_.start()
    x_cp(0).start(); u_cp(0).start()
    for c_ in par2_cps: c_.start()
    for i in range(1, 4):
        x_cp(i).start(); u_cp(i).start()
    g_cp.start(); wq_cp.start(); wo_cp.start(); wv_cp.start()
    for c_ in par_cps: c_.wait()

    def fence():
        pl.semaphore_signal(fsem, 1)
        pl.semaphore_wait(fsem, 1)

    dt_row = _rb(jnp.exp(ldt_ref[...].astype(f32).reshape(1, D)))
    dtb_ref[...] = jnp.broadcast_to(dt_row, (128, D)).T
    p_ref[...] = jnp.zeros_like(p_ref)
    zacc_ref[...] = jnp.zeros_like(zacc_ref)
    lane = lax.broadcasted_iota(jnp.int32, (8, 128), 1)

    def tables_pair(it, hh):
        r0 = pl.multiple_of(it * 32 + hh * 16, 16)
        rows = pl.ds(r0, 16)
        dtb = dtb_ref[rows, :]
        are, aim, bre, bim, cre, cim = [par_v[i, rows, :].astype(f32) for i in range(6)]
        zr_all = dtb * are; zi_all = dtb * aim
        wr_all, wi_all = _cmul(cre, cim, dtb * bre, dtb * bim)
        cur_it[0] = it
        return zr_all, zi_all, wr_all, wi_all

    cur_it = [None]
    def pre_rows(hh, h):
        return pl.ds(pl.multiple_of(cur_it[0] * 32 + hh * 16 + h * 8, 8), 8)

    def tables_g(par, hh, h, pre, tok=None):
        zr_all, zi_all, wr_all, wi_all = pre
        g = hh * 2 + h
        xt_ref = (xt0_ref, xt1_ref)[par]; yt_ref = (yt0_ref, yt1_ref)[par]
        zr = zr_all[8 * h:8 * h + 8]; zi = zi_all[8 * h:8 * h + 8]
        wr = wr_all[8 * h:8 * h + 8]; wi = wi_all[8 * h:8 * h + 8]
        zr = _dep_f32(zr, tok); zi = _dep_f32(zi, tok)
        low = lax.broadcasted_iota(jnp.int32, (8, 128), 0) < 4
        def mixA(x, y):
            return jnp.where(low, x, pltpu.roll(y, 4, 0))
        def mixB(x, y):
            return jnp.where(low, pltpu.roll(x, 4, 0), y)
        zrr = _rev8(zr); zir = _rev8(zi)
        e8 = _cexp(zrr, zir, -8.0, 8.0)
        ys = [None] * 32
        ys[0] = (jnp.ones_like(zr), jnp.zeros_like(zr))
        ys[1] = e8
        todo = [(ab, b2) for b2 in range(0, 16, 2) for ab in range(2)]
        def emit():
            for (ab, b2) in list(todo):
                off = 1 + ab
                idx = [(2 * b2 + off + k) % 32 for k in range(4)]
                if any(ys[i] is None for i in idx):
                    continue
                todo.remove((ab, b2))
                mix = (mixA, mixB)[ab]
                y_ = [ys[i] for i in idx]
                re = jnp.concatenate([mix(y_[0][0], y_[1][0]), mix(y_[2][0], y_[3][0])], 0).astype(bf16)
                im = jnp.concatenate([mix(y_[0][1], y_[1][1]), mix(y_[2][1], y_[3][1])], 0).astype(bf16)
                yt_ref[2 * g + ab, pl.ds(8 * b2, 16), 0:128] = re
                yt_ref[2 * g + ab, pl.ds(8 * b2, 16), 128:256] = im
        for lo in range(2, 32):
            ys[lo] = _cmul(*ys[lo - 1], *e8)
            emit()
        assert not todo
        tk_ = _tok(ys[31][0])
        zr = _dep_f32(zr, tk_); zi = _dep_f32(zi, tk_)
        e1 = _cexp(zr, zi, 1.0)
        e2 = _cmul(*e1, *e1)
        e4 = _cmul(*e2, *e2)
        sm = {2: e2, 4: e4, 6: _cmul(*e4, *e2)}
        e256 = _cexp(zr, zi, 256.0)
        slots = {}
        for si, hv in enumerate(_HI):
            slots.setdefault(int(hv) // 256, []).append((si, int(hv) % 256))
        q = (wr, wi)
        pend = {}
        for a in range(9):
            if a > 0:
                q = _cmul(*q, *e256)
            prev = q
            for (si, c) in slots.get(a, []):
                if c == 0:
                    pend[si] = q
                elif a == 0:
                    prev = _cmul(*prev, *e1)
                    pend[si] = prev
                else:
                    pend[si] = _cmul(*q, *sm[c])
                s0 = si & ~3
                if all(s0 + k in pend for k in range(4)):
                    e = [pend.pop(s0 + k) for k in range(4)]
                    for (gg, mix) in ((2 * g, mixA), (2 * g + 1, mixB)):
                        re = jnp.concatenate([mix(e[0][0], e[1][0]), mix(e[2][0], e[3][0])], 0).astype(bf16)
                        im = jnp.concatenate([mix(e[0][1], e[1][1]), mix(e[2][1], e[3][1])], 0).astype(bf16)
                        xt_ref[gg, pl.ds(4 * s0, 16), 0:128] = re
                        xt_ref[gg, pl.ds(4 * s0, 16), 128:256] = im
        assert not pend
        r0 = pre_rows(hh, h)
        k2048_ref[r0, :] = jnp.broadcast_to(jnp.sum(q[0], axis=1, keepdims=True), (8, 128))
        tk2 = _tok(q[1] + ys[31][0])
        for _i in range(DEL[g]):
            tk2 = pltpu.roll(tk2, 1, 1)
        return tk2

    def tables(it, par):
        for hh in range(2):
            pre = tables_pair(it, hh)
            for h in range(2):
                tables_g(par, hh, h, pre)

    def kgen_pair(it, par, hh):
        parts = []
        xt_ref = (xt0_ref, xt1_ref)[par]; yt_ref = (yt0_ref, yt1_ref)[par]
        low = lax.broadcasted_iota(jnp.int32, (8, 128), 0) < 4
        for h in range(2):
            g = hh * 2 + h
            oa = _nt(xt_ref[2 * g], yt_ref[2 * g])
            ob = _nt(xt_ref[2 * g + 1], yt_ref[2 * g + 1])
            merged = []
            for m in range(5):
                acc = None
                for pp in range(2):
                    p = 2 * m + pp
                    A_ = oa[8 * p:8 * p + 8, :]; B_ = ob[8 * p:8 * p + 8, :]
                    S0 = jnp.where(low, A_, pltpu.roll(B_, 4, 0))
                    S1 = jnp.where(low, pltpu.roll(A_, 4, 0), B_)
                    for e, S in enumerate((S0, S1)):
                        c = 2 * pp + e
                        rolled = pltpu.roll(S, c + 1, 1, stride=1, stride_axis=0)
                        acc = rolled if acc is None else jnp.where((lane & 3) == c, rolled, acc)
                merged.append(acc)
            P, Q = merged[0], merged[1]
            tA = jnp.where(lane < 64, P, pltpu.roll(Q, 64, 1))
            tB = jnp.where(lane < 64, pltpu.roll(P, 64, 1), Q)
            k2 = k2048_ref[pl.ds(pl.multiple_of(it * 32 + hh * 16 + h * 8, 8), 8), :]
            parts.append(jnp.concatenate([tA, tB, merged[2], merged[3], merged[4], jnp.where(lane == 0, k2, 0.0)], 1))
        r0 = pl.multiple_of(it * 16 + hh * 8, 8)
        kt_ref[pl.ds(r0, 8), :] = _pk(jnp.concatenate(parts, 0).astype(bf16))

    def kgen(it, par):
        kgen_pair(it, par, 0); kgen_pair(it, par, 1)

    def b_k(it):
        rows = pl.ds(pl.multiple_of(it * C, C), C)
        kT = _nt(_up(wkt_ref[...]), x_v[rows, :])
        pkf = _phi(kT)
        zacc_ref[...] += pkf
        return pkf.astype(bf16)

    def b_p(pkT, it):
        rows = pl.ds(pl.multiple_of(it * C, C), C)
        p_ref[...] += _nn(pkT, x_v[rows, :])

    def ufwd(a, par):
        uf = _nn(_up(f_ref[...]), u_v[pl.ds(pl.multiple_of(a * C, C), C), :])
        ar, ai = uf[:128], uf[128:]
        cur = (ur0_ref, ur1_ref)[par]; prv = (ur0_ref, ur1_ref)[1 - par]
        cur[...] = uf
        if not (isinstance(a, int) and a == 0):
            pr = prv[0:128, :]; pi_ = prv[128:256, :]
            ar, ai = (jnp.concatenate([ar[:64] - pi_[:64], ar[64:] + pi_[64:]], 0),
                      jnp.concatenate([ai[:64] + pr[:64], ai[64:] - pr[64:]], 0))
        for t in range(4):
            ln = slice(t * 128, (t + 1) * 128)
            pu_ref[t, 0, a] = ar[:, ln]
            pu_ref[t, 1, a] = ai[:, ln]
            pu_ref[t, 2, a] = ar[:, ln] + ai[:, ln]

    tables(0, 0)
    for c_ in xu0_cps: c_.wait()
    for c_ in f_cps: c_.wait()
    ufwd(0, 0)
    wk_cp.wait()
    wkt_ref[...] = _pk(w_v[:, D:2 * D].astype(f32).T.astype(bf16))
    b_p(b_k(0), 0)
    x_cp(0).wait(); u_cp(0).wait()

    def step1(it, par):
        pkT = b_k(it)
        pre = tables_pair(it, 0)
        t1 = tables_g(par, 0, 0, pre)
        t2 = tables_g(par, 0, 1, pre, t1)
        kgen_pair(it - 1, 1 - par, 0)
        ufwd(it, par)
        pre = tables_pair(it, 1)
        t3 = tables_g(par, 1, 0, pre, t2)
        kgen_pair(it - 1, 1 - par, 1)
        tables_g(par, 1, 1, pre, t3)
        b_p(pkT, it)

    step1(1, 1)
    def body1(i2, carry):
        @pl.when(i2 % 2 == 0)
        def _():
            x_cp(i2 // 2).wait(); u_cp(i2 // 2).wait()
        @pl.when(i2 == 2)
        def _():
            for c_ in par2_cps: c_.wait()
        step1(2 * i2, 0)
        fence()
        step1(2 * i2 + 1, 1)
        return carry
    lax.fori_loop(1, NC // 2, body1, 0)
    kgen(NC - 1, 1)

    g_cp.wait(); wo_cp.wait(); wq_cp.wait(); wv_cp.wait()
    wqp_ref[...] = _pk(w_v[:, 0:D])
    def kf(t, r4, jj):
        pk_ref = (pk0_ref, pk1_ref)[t % 2]
        j = _sel(r4, _SLOT_J[jj])
        t0 = _sel(r4, _SLOT_T0[jj])
        rows = slice(t * 64, (t + 1) * 64)
        def lanes(k):
            if isinstance(t0, int):
                return slice((t0 + k) * 128, (t0 + k + 1) * 128)
            return pl.ds(pl.multiple_of((t0 + k) * 128, 128), 128)
        if jj == 0:
            kf_ = _nt(_up(g_v[2 * r4]), _up(kt_ref[rows, lanes(0)])) + _nt(_up(g_v[2 * r4 + 1]), _up(kt_ref[rows, lanes(1)]))
        else:
            kf_ = _nt(_up(g_v[8 + (jj - 1) * 4 + r4]), _up(kt_ref[rows, lanes(0)]))
        c_, d_ = kf_[:128], kf_[128:]
        pk_ref[0, j] = c_
        pk_ref[1, j] = d_ - c_
        pk_ref[2, j] = c_ + d_

    for r4 in range(4):
        for jj in range(4):
            kf(0, r4, jj)

    zcol = _rb(jnp.sum(zacc_ref[...], axis=1, keepdims=True))
    ri = lax.broadcasted_iota(jnp.int32, (128, 128), 0) // 16
    ci = lax.broadcasted_iota(jnp.int32, (128, 128), 1) // 16
    bm = ri == ci
    for g in range(4):
        zm_ref[g] = _pk(jnp.where(bm, jnp.broadcast_to(zcol[g * 128:(g + 1) * 128], (128, 128)), 0.0).astype(bf16))
        kvg = _nn(p_ref[g * 128:(g + 1) * 128, :].astype(bf16), w_v[:, 2 * D + g * 128:2 * D + (g + 1) * 128])
        kvm = jnp.where(bm, kvg, 0.0).astype(bf16)
        mm_ref[g * 64:(g + 1) * 64, :] = _pk(_nn(kvm, wo_v[g * 128:(g + 1) * 128, :]).astype(bf16))

    dsk_ref2[...] = jnp.broadcast_to(dsk_ref[...].astype(f32).reshape(1, D), (8, D))

    def conv_pos(rg, t, token):
        z_ref = (z0_ref, z1_ref)[t % 2]
        pk_ref = (pk0_ref, pk1_ref)[t % 2]
        rows = pl.ds(pl.multiple_of(rg * 8, 8), 8)
        rows_im = pl.ds(pl.multiple_of(128 + rg * 8, 8), 8)
        for ps in range(2):
            U = {i: tuple(pu_ref[t, m, i, rows, :] for m in range(3)) for i in range(8 * ps, 8 * ps + 8)}
            for a in range(8 * ps, NC):
                acc = None
                for i in range(8 * ps, min(a, 8 * ps + 7) + 1):
                    j = a - i
                    kc = pk_ref[0, j, rows, :]; kdc = pk_ref[1, j, rows, :]; kcd = pk_ref[2, j, rows, :]
                    ua, ub, uab = U[i]
                    t1 = kc * uab; t2 = ua * kdc; t3 = ub * kcd
                    if acc is None:
                        if token is not None:
                            t1 = t1 + token
                        acc = [t1, t2, t3]
                    else:
                        acc = [acc[0] + t1, acc[1] + t2, acc[2] + t3]
                zr_ = acc[0] - acc[2]
                zi_ = acc[0] + acc[1]
                if ps == 1:
                    zr_ = zr_ + z_ref[a, rows, :]
                    zi_ = zi_ + z_ref[a, rows_im, :]
                z_ref[a, rows, :] = zr_
                z_ref[a, rows_im, :] = zi_
                token = jnp.minimum(jnp.abs(zr_), 0.0) if TOK[t] else (zr_ - zr_)
        return token

    def bout(i):
        rows = pl.ds(pl.multiple_of(i * C, C), C)
        xc = x_v[rows, :]
        q = _nn(xc, _up(wqp_ref[...]))
        pq = _phi(q)
        pqb = pq.astype(bf16)
        den = jnp.concatenate([_nn(pqb[:, g * 128:(g + 1) * 128], _up(zm_ref[g])) for g in range(4)], 1) + 1e-6
        pp = (pq * _recip(den)).astype(bf16)
        ob_v[rows, :] = _nn(pp, _up(mm_ref[...])).astype(bf16)
        ob_cp(i).start()

    def ob_cp(i):
        rows = pl.ds(pl.multiple_of(i * C, C), C)
        return cp(ob_v.at[rows, :], o_hbm.at[rows, D:2 * D], sems.at[S_OB])

    def oa_cp(t, r4):
        rows = pl.ds(pl.multiple_of(r4 * 512, 512), 512)
        return cp(oa_v.at[t, rows, :], o_hbm.at[rows, t * 128:(t + 1) * 128], sems.at[S_OA])

    def inv(t, r4):
        z_ref = (z0_ref, z1_ref)[t % 2]
        lanes = slice(t * 128, (t + 1) * 128)
        for aa in range(4):
            a = r4 * 4 + aa
            rows = pl.ds(pl.multiple_of(a * C, C), C)
            y = _nn(_up(fi_ref[...]), z_ref[a].astype(bf16))
            oa_v[t, rows, :] = (y + u_v[rows, lanes].astype(f32) * dsk_ref2[0:1, lanes]).astype(bf16)
        oa_cp(t, r4).start()

    def body3(t, r4):
        token = None
        bout(t * 4 + r4)
        if t > 0:
            inv(t - 1, r4)
        if t < 3:
            for jj in range(4):
                kf(t + 1, r4, jj)
        for p in range(4):
            token = conv_pos(r4 * 4 + p, t, token)

    for t in range(4):
        def b3(r4, carry, t=t):
            body3(t, r4)
            return carry
        lax.fori_loop(0, 4, b3, 0)
    for r4 in range(4):
        inv(3, r4)
    cp(ob_v, o_hbm.at[:, D:2 * D], sems.at[S_OB]).wait()
    cp(ob_v, o_hbm.at[:, 0:D], sems.at[S_OA]).wait()


TOK = (0, 1, 1, 0)
DEL = (1, 1, 1, 0)


@jax.jit
def pallas_concat_heads__ssm_conv_s4__linear_attn_block__prompt_kernel(
        A_u, A_A_re, A_A_im, A_B_re, A_B_im, A_C_re, A_C_im, A_log_dt, A_Dskip, B_x, B_wqkv, B_wo):
    u = A_u.reshape(L, D)
    x = B_x.reshape(L, D)
    F = jnp.asarray(_pack_np(_F)); FI = jnp.asarray(_pack_np(_FI)); G = jnp.asarray(_pack_np(_G))
    anyspec = pl.BlockSpec(memory_space=pl.ANY)
    out = pl.pallas_call(
        kernel,
        out_shape=jax.ShapeDtypeStruct((L, 2 * D), bf16),
        in_specs=[anyspec] * 15,
        out_specs=anyspec,
        scratch_shapes=[
            pltpu.SemaphoreType.DMA((NSEM,)),
            pltpu.SemaphoreType.REGULAR,
            pltpu.VMEM((D, D), f32),
            pltpu.VMEM((D,), bf16), pltpu.VMEM((D,), bf16), pltpu.VMEM((128, 128), u32), pltpu.VMEM((64, 256), u32),
            pltpu.VMEM((6, D, N), bf16),
            pltpu.VMEM((L, D), bf16),
            pltpu.VMEM((L, D), bf16),
            pltpu.VMEM((D, 3 * D), bf16),
            pltpu.VMEM((D, D), bf16),
            pltpu.VMEM((NGT, 128, 128), u32),
            pltpu.VMEM((4, L, 128), bf16),
            pltpu.VMEM((L, D), bf16),
            pltpu.VMEM((D, 128), f32),
            pltpu.VMEM((8, 4 * NHI, 256), bf16),
            pltpu.VMEM((8, 4 * NHI, 256), bf16),
            pltpu.VMEM((8, 128, 256), bf16),
            pltpu.VMEM((8, 128, 256), bf16),
            pltpu.VMEM((D // 2, 768), u32),
            pltpu.VMEM((3, NC, 128, 128), f32),
            pltpu.VMEM((3, NC, 128, 128), f32),
            pltpu.VMEM((4, 3, NC, 128, 128), f32),
            pltpu.VMEM((NC, 256, 128), f32),
            pltpu.VMEM((NC, 256, 128), f32),
            pltpu.VMEM((D // 2, D), u32),
            pltpu.VMEM((D, 128), f32),
            pltpu.VMEM((4, 64, 128), u32),
            pltpu.VMEM((D // 2, D), u32),
            pltpu.VMEM((8, D), f32),
            pltpu.VMEM((D // 2, D), u32),
            pltpu.VMEM((256, D), f32),
            pltpu.VMEM((256, D), f32),
            pltpu.VMEM((D, 128), f32),
        ],
        compiler_params=pltpu.CompilerParams(vmem_limit_bytes=110 * 1024 * 1024),
    )(u, A_A_re, A_A_im, A_B_re, A_B_im, A_C_re, A_C_im, A_log_dt, A_Dskip, x, B_wqkv, B_wo, F, FI, G)
    return out.reshape(1, L, 2 * D)
```
